```python
import os as _os
_os.environ.setdefault("JAX_PLATFORMS", "cpu")
import jax
import jax.numpy as jnp

def _softmax(x, axis=-1):
    return jax.nn.softmax(x, axis=axis)
def _gelu(x):
    return jax.nn.gelu(x, approximate=True)
def _silu(x):
    return jax.nn.silu(x)
def _sigmoid(x):
    return jax.nn.sigmoid(x)
def _layernorm(x, axis=-1, eps=1e-5):
    m = jnp.mean(x, axis=axis, keepdims=True)
    v = jnp.var(x, axis=axis, keepdims=True)
    return (x - m) / jnp.sqrt(v + eps)
def _scatter_add(tgt, idx, src, axis=0):
    return tgt.at[idx].add(src)
def _segment_sum(src, seg, n):
    return jax.ops.segment_sum(src, seg, n)
class _Rng:
    def __init__(self, key):
        self._k = key
    def _next(self):
        self._k, sub = jax.random.split(self._k)
        return sub
    def normal(self, shape):
        return jax.random.normal(self._next(), shape, dtype=jnp.bfloat16)
    def randint(self, lo, hi, shape):
        return jax.random.randint(self._next(), shape, lo, hi, dtype=jnp.int32)
    def uniform(self, shape, lo=0.0, hi=1.0):
        return jax.random.uniform(self._next(), shape, jnp.bfloat16, lo, hi)
    def permutation(self, n):
        return jax.random.permutation(self._next(), n)


kernel_name = 'interleave_layers__sliding_local_dilated__linear_kernel_hedgehog__prompt'

def setup_inputs():
    _rng = _Rng(jax.random.key(int.from_bytes(__import__("os").urandom(4), "little")))
    _w = (lambda a: (lambda t: t.astype(jnp.bfloat16) if jnp.issubdtype(t.dtype, jnp.floating) else t)(jnp.asarray(a)))
    def _A_setup():
        B, S, D = 1, 2048, 640
        return {
            "x": _w((lambda *s: _rng.normal(s) * 0.05)(B, S, D)),
            "wqkv": _w((lambda *s: _rng.normal(s) * 0.05)(D, 3 * D)),
            "wo": _w((lambda *s: _rng.normal(s) * 0.05)(D, D)),
        }
    _A_in = _A_setup()

    def _B_setup():
        B, S, D, H = 1, 2048, 640, 32
        Dh = D // H
        return {
            "x": _w((lambda *s: _rng.normal(s) * 0.05)(B, S, D)),
            "wqkv": _w((lambda *s: _rng.normal(s) * 0.4)(D, 3 * D)),
            "w_phi": _w((lambda *s: _rng.normal(s) * 0.4)(H, Dh, Dh) * (Dh ** -0.5)),
            "wo": _w((lambda *s: _rng.normal(s) * 0.1)(D, D)),
        }
    _B_in = _B_setup()

    return {
        "A_x": _A_in["x"],
        "A_wqkv": _A_in["wqkv"],
        "A_wo": _A_in["wo"],
        "B_x": _B_in["x"],
        "B_wqkv": _B_in["wqkv"],
        "B_w_phi": _B_in["w_phi"],
        "B_wo": _B_in["wo"],
    }

def reference(A_x, A_wqkv, A_wo, B_x, B_wqkv, B_w_phi, B_wo):
    def _A_ref(x, wqkv, wo):
        B, S, D = x.shape
        H = 32; Dh = D // H
        W, dil = 8, 2
        qkv = (lambda x, *d: x.transpose(*d))((x @ wqkv).reshape(B, S, 3, H, Dh), 2, 0, 3, 1, 4)
        q, k, v = qkv[0], qkv[1], qkv[2]
        scale = Dh ** -0.5
        pos = jnp.arange(S)
        off = jnp.arange(W) * dil
        idx = pos[:, None] - off[None, :]
        mask = idx >= 0
        idx_c = jnp.where(mask, idx, 0).reshape(-1)
        kg = k[:, :, idx_c, :].reshape(B, H, S, W, Dh)
        vg = v[:, :, idx_c, :].reshape(B, H, S, W, Dh)
        logits = jnp.einsum("bhsd,bhswd->bhsw", q, kg) * scale
        logits = jnp.where(mask[None, None, :, :], logits, -1e9)
        attn = _softmax(logits, axis=-1)
        o = jnp.einsum("bhsw,bhswd->bhsd", attn, vg)
        return (lambda x, *d: x.transpose(*d))(o, 0, 2, 1, 3).reshape(B, S, D) @ wo

    def _B_ref(x, wqkv, w_phi, wo):
        B, S, D = x.shape
        H = 32; Dh = D // H
        qkv = (lambda x, *d: x.transpose(*d))((x @ wqkv).reshape(B, S, 3, H, Dh), 2, 0, 3, 1, 4)
        q, k, v = qkv[0], qkv[1], qkv[2]
        pq = jnp.einsum("bhsd,hdf->bhsf", q, w_phi)
        pk = jnp.einsum("bhsd,hdf->bhsf", k, w_phi)
        phi_q = jnp.concatenate([_softmax(pq, axis=-1), _softmax(-pq, axis=-1)], axis=-1)
        phi_k = jnp.concatenate([_softmax(pk, axis=-1), _softmax(-pk, axis=-1)], axis=-1)
        kv = jnp.einsum("bhsf,bhsd->bhfd", phi_k, v)
        z  = jnp.einsum("bhsf->bhf", phi_k)
        num = jnp.einsum("bhqf,bhfd->bhqd", phi_q, kv)
        den = jnp.einsum("bhqf,bhf->bhq", phi_q, z)[..., None] + 1e-6
        o = num / den
        return (lambda x, *d: x.transpose(*d))(o, 0, 2, 1, 3).reshape(B, S, D) @ wo

    x = A_x
    x = x + _A_ref(_layernorm(x, axis=-1), A_wqkv, A_wo)
    x = x + _B_ref(_layernorm(x, axis=-1), B_wqkv, B_w_phi, B_wo)
    x = x + _A_ref(_layernorm(x, axis=-1), A_wqkv, A_wo)
    x = x + _B_ref(_layernorm(x, axis=-1), B_wqkv, B_w_phi, B_wo)
    return x
```

```python
import jax
import jax.numpy as jnp
import numpy as np
import jax.experimental.pallas as pl
import jax.experimental.pallas.tpu as pltpu

S, D, H, DH = 2048, 640, 32, 20
W, DIL = 8, 2
MC = 256
NC = 256
HALO = 16
NA, NB = S // MC, S // NC
LOG2E = float(np.log2(np.e))
bf16, f32 = jnp.bfloat16, jnp.float32
NT = (((1,), (1,)), ((), ()))


def _dot(a, b):
    return jnp.dot(a, b, preferred_element_type=f32)


def _dot_nt(a, b):
    return jax.lax.dot_general(a, b, NT, preferred_element_type=f32)


def _ln(x):
    m = jnp.sum(x, axis=-1, keepdims=True) * (1.0 / D)
    d = x - m
    v = jnp.sum(d * d, axis=-1, keepdims=True) * (1.0 / D)
    return d * jax.lax.rsqrt(v + 1e-5)


def _rcp(x):
    r = pl.reciprocal(x, approx=True)
    return r * (2.0 - x * r)


def _tree(op, xs):
    xs = list(xs)
    while len(xs) > 1:
        nx = [op(xs[i], xs[i + 1]) for i in range(0, len(xs) - 1, 2)]
        if len(xs) % 2:
            nx.append(xs[-1])
        xs = nx
    return xs[0]


def kernel(x_hbm, awqkv_hbm, awo_hbm, bwqkv_hbm, wphi_hbm, bwo_hbm, out_hbm,
           xin, wraw, woraw, wphi, w2,
           awt, awo, bwt, bwo,
           xs, xh, ob,
           q, k, v, kh, vh, o,
           pt, vloc, phik, phiq, kvacc, kvl, ot,
           sems):
    cp_aw = pltpu.make_async_copy(awqkv_hbm, wraw.at[0], sems.at[0])
    cp_x = pltpu.make_async_copy(x_hbm, xin, sems.at[1])
    cp_ao = pltpu.make_async_copy(awo_hbm, woraw.at[0], sems.at[2])
    cbw = [pltpu.make_async_copy(bwqkv_hbm.at[:, pl.ds(D * b, D)], wraw.at[1, :, pl.ds(D * b, D)], sems.at[m])
           for b, m in enumerate((3, 6 + NB, 7 + NB))]
    cp_ph = pltpu.make_async_copy(wphi_hbm, wphi, sems.at[4])
    cp_bo = pltpu.make_async_copy(bwo_hbm, woraw.at[1], sems.at[5])
    for c in (cbw[0], cp_ph, cbw[1], cp_bo, cbw[2], cp_ao, cp_x, cp_aw):
        c.start()

    row = jax.lax.broadcasted_iota(jnp.int32, (160, 256), 0)
    col = jax.lax.broadcasted_iota(jnp.int32, (160, 256), 1)
    rd, rh = row >> 3, row & 7

    def perm(g):
        return (col == 32 * g + DH * rh + rd).astype(f32).astype(bf16)

    cp_ph.wait()
    lane = jax.lax.broadcasted_iota(jnp.int32, (DH, 128), 1)
    w2[...] = jnp.zeros(w2.shape, f32)
    for h in range(H):
        w2[pl.ds(DH * h, DH), pl.ds(0, DH)] = wphi[h].astype(f32)
    er = jax.lax.broadcasted_iota(jnp.int32, (160, 128), 0)
    ec = jax.lax.broadcasted_iota(jnp.int32, (160, 128), 1)
    emat = ((er >> 3) == ec).astype(f32).astype(bf16)
    phis = []
    for g in range(4):
        t = _dot_nt(emat, w2[pl.ds(128 * g, 256), :].astype(bf16))
        u = col - 32 * g - DH * rh
        phis.append(jnp.where(jnp.logical_and(u >= 0, u < DH), t, 0.0).astype(bf16))
    for b in range(3):
        cbw[b].wait()
        for g in range(4):
            r = _dot_nt(phis[g] if b < 2 else perm(g), wraw[1, :, pl.ds(D * b + 128 * g, 256)])
            r = r * LOG2E if b < 2 else r
            bwt[pl.ds(D * (2 - b) + 160 * g, 160), :] = r.astype(bf16)
    cp_bo.wait(); cp_ao.wait()
    for j in range(2):
        for t in range(5):
            cs = pl.ds(128 * t, 128)
            w2[...] = woraw[j, :, cs].astype(f32)
            for d in range(DH):
                for gp in range(2):
                    dst = (awo, bwo)[j]
                    if j == 0:
                        dst[pl.ds(32 * d + 16 * gp, 16), cs] = w2[pl.ds(320 * gp + d, 16, stride=DH), :].astype(bf16)
                    else:
                        for g in (2 * gp, 2 * gp + 1):
                            if d % 2 == 0:
                                val = [w2[pl.ds(160 * g + e, 8, stride=DH), :] for e in (d, d + 1)]
                                dst[pl.ds(160 * g + 8 * d, 16), cs] = jnp.concatenate(val, axis=0).astype(bf16)
    cp_aw.wait()
    for gp in range(2):
        p0, p1 = perm(2 * gp), perm(2 * gp + 1)
        for b in range(3):
            if b < 3:
                r0 = _dot_nt(p0, wraw[0, :, pl.ds(D * b + 128 * (2 * gp), 256)])
                r1 = _dot_nt(p1, wraw[0, :, pl.ds(D * b + 128 * (2 * gp + 1), 256)])
            else:
                r0 = _dot(p0, woraw[0, pl.ds(128 * (2 * gp), 256), :])
                r1 = _dot(p1, woraw[0, pl.ds(128 * (2 * gp + 1), 256), :])
            if b == 0:
                r0 = r0 * (LOG2E * DH ** -0.5)
                r1 = r1 * (LOG2E * DH ** -0.5)
            for d in range(DH):
                val = jnp.concatenate([r0[8 * d:8 * d + 8], r1[8 * d:8 * d + 8]], axis=0).astype(bf16)
                if b < 3:
                    awt[pl.ds(D * b + 32 * d + 16 * gp, 16), :] = val
                else:
                    awo[pl.ds(32 * d + 16 * gp, 16), :] = val

    phik[:, :, pl.ds(320, 64), :] = jnp.zeros((2, 4, 64, NC), bf16)
    for c in range(S // NC):
        phiq[c, :, pl.ds(320, 64), :] = jnp.zeros((4, 64, NC), bf16)
    vloc[:, :, pl.ds(160, 16), :] = jnp.ones((2, 4, 16, NC), bf16)

    cp_x.wait()

    def ln0(i, _):
        r = pl.ds(pl.multiple_of(i * MC, MC), MC)
        x = xin[r, :].astype(f32)
        xs[r, :] = x
        xh[r, :] = _ln(x).astype(bf16)
    jax.lax.fori_loop(0, S // MC, ln0, None)

    def qkv(c, bs=(0, 1, 2)):
        i = c % 2
        for b in bs:
            r = _dot_nt(xh[pl.ds(c * MC, MC), :], awt[pl.ds(D * b, D), :])
            for t in range(5):
                rt = r[:, 128 * t:128 * t + 128]
                if b == 0:
                    q[i, t] = rt
                    continue
                d, h = ((k, kh), (v, vh))[b - 1]
                d[i, t, pl.ds(HALO, MC), :] = rt
                if c + 1 < NA:
                    h[(c + 1) % 3, t] = rt[MC - HALO:]
                if c == 0:
                    d[0, t, pl.ds(0, HALO), :] = jnp.zeros((HALO, 128), f32)

    def att(c, part):
        i = c % 2
        RG = 8
        prev = {}
        if c > 0 and part == 0:
            k[i, :, pl.ds(0, HALO), :] = kh[c % 3]
            v[i, :, pl.ds(0, HALO), :] = vh[c % 3]
        for rg in range(8 * part, 8 * part + 8):
            r0 = rg * RG
            acc5 = []
            qs = [q[i, t, pl.ds(r0, RG), :] for t in range(5)]
            ls = []
            for w in range(W):
                s = _tree(jnp.add, [qs[t] * k[i, t, pl.ds(HALO + r0 - DIL * w, RG), :] for t in range(5)])
                s = s + pltpu.roll(s, 64, 1)
                s = s + pltpu.roll(s, 32, 1)
                if c == 0 and r0 < DIL * w:
                    pos = r0 + jax.lax.broadcasted_iota(jnp.int32, (RG, 128), 0)
                    s = jnp.where(pos >= DIL * w, s, -1e9)
                ls.append(s)
            m = _tree(jnp.maximum, ls)
            ps = [jnp.exp2(s - m) for s in ls]
            inv = _rcp(_tree(jnp.add, ps))
            for t in range(5):
                acc = _tree(jnp.add, [ps[w] * v[i, t, pl.ds(HALO + r0 - DIL * w, RG), :] for w in range(W)])
                acc = acc * inv
                if rg % 2 == 0:
                    prev[t] = acc
                else:
                    o[i, pl.ds(r0 - RG, 16), pl.ds(128 * t, 128)] = jnp.concatenate([prev[t], acc], axis=0).astype(bf16)

    def proj(c):
        r = pl.ds(c * MC, MC)
        x = xs[r, :] + _dot(o[c % 2], awo[...])
        xs[r, :] = x
        xh[r, :] = _ln(x).astype(bf16)

    def bmm(c):
        i = c % 2
        r = _dot_nt(bwt[...], xh[pl.ds(c * NC, NC), :])
        pt[i] = r[D:]
        for g in range(4):
            vloc[i, g, pl.ds(0, 160), :] = r[160 * g:160 * g + 160].astype(bf16)

    def soft(c):
        i = c % 2
        for off in (0, D):
            for g in range(4):
                for ct in range(NC // 128):
                    cs = pl.ds(128 * ct, 128)
                    p = [pt[i, pl.ds(off + 160 * g + 8 * f, 8), cs] for f in range(DH)]
                    mx = _tree(jnp.maximum, p)
                    mn = _tree(jnp.minimum, p)
                    ep = [jnp.exp2(a - mx) for a in p]
                    ip = _rcp(_tree(jnp.add, ep))
                    en = [jnp.exp2(mn - a) for a in p]
                    im = _rcp(_tree(jnp.add, en))
                    for f in range(DH):
                        val = jnp.concatenate([ep[f] * ip, en[f] * im], axis=0).astype(bf16)
                        if off == 0:
                            phik[i, g, pl.ds(16 * f, 16), cs] = val
                        else:
                            phiq[c, g, pl.ds(16 * f, 16), cs] = val

    def kvmm(c):
        i = c % 2
        for g in range(4):
            r = _dot_nt(vloc[i, g], phik[i, g])
            kvacc[g] = r if c == 0 else kvacc[g] + r

    def kvfin():
        kr = jax.lax.broadcasted_iota(jnp.int32, (176, 384), 0)
        kc = jax.lax.broadcasted_iota(jnp.int32, (176, 384), 1)
        for g in range(4):
            kvl[g] = jnp.where((kr & 7) == (kc & 7), kvacc[g], 0.0).astype(bf16)

    def one(c):
        for g in range(4):
            r = _dot(kvl[g], phiq[c, g])
            inv = _rcp(r[160:168] + 1e-6)
            for d in range(DH):
                ot[c % 2, pl.ds(160 * g + 8 * d, 8), :] = r[8 * d:8 * d + 8] * inv

    def ocopy(c):
        r = pl.ds(c * NC, NC)
        return pltpu.make_async_copy(ob.at[r], out_hbm.at[r], sems.at[6 + c])

    def two(c):
        oo = ot[c % 2].T.astype(bf16)
        r = pl.ds(c * NC, NC)
        x = xs[r, :] + _dot(oo, bwo[...])
        xs[r, :] = x
        xh[r, :] = _ln(x).astype(bf16)
        ob[r, :] = x.astype(bf16)
        ocopy(c).start()

    def pair(l, _):
        qkv(0)
        for c in range(NA):
            if c > 0:
                proj(c - 1)
            att(c, 0)
            for b in range(3):
                if c + 1 < NA:
                    qkv(c + 1, (b,))
                att(c, b + 1)
        proj(NA - 1)
        bmm(0)
        for c in range(NB):
            if c > 0:
                kvmm(c - 1)
            if c + 1 < NB:
                bmm(c + 1)
            soft(c)
        kvmm(NB - 1)

        @pl.when(l > 0)
        def _():
            for c in range(NB):
                ocopy(c).wait()
        kvfin()
        one(0)
        for c in range(NB):
            if c + 1 < NB:
                one(c + 1)
            two(c)
    jax.lax.fori_loop(0, 2, pair, None)
    for c in range(NB):
        ocopy(c).wait()


@jax.jit
def pallas_interleave_layers__sliding_local_dilated__linear_kernel_hedgehog__prompt_kernel(
        A_x, A_wqkv, A_wo, B_x, B_wqkv, B_w_phi, B_wo):
    del B_x
    V = pltpu.VMEM
    scratch = [
        V((S, D), bf16), V((2, D, 3 * D), bf16), V((2, D, D), bf16), V((H, DH, DH), bf16), V((D, 128), f32),
        V((3 * D, D), bf16), V((D, D), bf16), V((3 * D, D), bf16), V((D, D), bf16),
        V((S, D), f32), V((S, D), bf16), V((S, D), bf16),
        V((2, 5, MC, 128), f32), V((2, 5, MC + HALO, 128), f32), V((2, 5, MC + HALO, 128), f32),
        V((3, 5, HALO, 128), f32), V((3, 5, HALO, 128), f32), V((2, MC, D), bf16),
        V((2, 2 * D, NC), f32), V((2, 4, 176, NC), bf16), V((2, 4, 384, NC), bf16),
        V((S // NC, 4, 384, NC), bf16), V((4, 176, 384), f32), V((4, 176, 384), bf16), V((2, D, NC), f32),
        pltpu.SemaphoreType.DMA((8 + NB,)),
    ]
    hbm = pl.BlockSpec(memory_space=pl.ANY)
    out = pl.pallas_call(
        kernel,
        out_shape=jax.ShapeDtypeStruct((S, D), bf16),
        in_specs=[hbm] * 6,
        out_specs=hbm,
        scratch_shapes=scratch,
        compiler_params=pltpu.CompilerParams(vmem_limit_bytes=110 * 2 ** 20),
    )(A_x.reshape(S, D), A_wqkv, A_wo, B_wqkv, B_w_phi, B_wo)
    return out.reshape(1, S, D)
```
